```python
import os as _os
_os.environ.setdefault("JAX_PLATFORMS", "cpu")
import jax
import jax.numpy as jnp

def _softmax(x, axis=-1):
    return jax.nn.softmax(x, axis=axis)
def _gelu(x):
    return jax.nn.gelu(x, approximate=True)
def _silu(x):
    return jax.nn.silu(x)
def _sigmoid(x):
    return jax.nn.sigmoid(x)
def _layernorm(x, axis=-1, eps=1e-5):
    m = jnp.mean(x, axis=axis, keepdims=True)
    v = jnp.var(x, axis=axis, keepdims=True)
    return (x - m) / jnp.sqrt(v + eps)
def _scatter_add(tgt, idx, src, axis=0):
    return tgt.at[idx].add(src)
def _segment_sum(src, seg, n):
    return jax.ops.segment_sum(src, seg, n)
class _Rng:
    def __init__(self, key):
        self._k = key
    def _next(self):
        self._k, sub = jax.random.split(self._k)
        return sub
    def normal(self, shape):
        return jax.random.normal(self._next(), shape, dtype=jnp.bfloat16)
    def randint(self, lo, hi, shape):
        return jax.random.randint(self._next(), shape, lo, hi, dtype=jnp.int32)
    def uniform(self, shape, lo=0.0, hi=1.0):
        return jax.random.uniform(self._next(), shape, jnp.bfloat16, lo, hi)
    def permutation(self, n):
        return jax.random.permutation(self._next(), n)


kernel_name = 'sequential_preLN__sliding_block__dense_activation_relu__prompt'

def setup_inputs():
    _rng = _Rng(jax.random.key(int.from_bytes(__import__("os").urandom(4), "little")))
    _w = (lambda a: (lambda t: t.astype(jnp.bfloat16) if jnp.issubdtype(t.dtype, jnp.floating) else t)(jnp.asarray(a)))
    def _A_setup():
        B, S, D = 1, 2048, 640
        return {
            "x": _w((lambda *s: _rng.normal(s) * 0.05)(B, S, D)),
            "wqkv": _w((lambda *s: _rng.normal(s) * 0.05)(D, 3 * D)),
            "wo": _w((lambda *s: _rng.normal(s) * 0.05)(D, D)),
        }
    _A_in = _A_setup()

    def _B_setup():
        B, S, D, Dff = 1, 2048, 640, 1536
        return {
            "x": _w((lambda *s: _rng.normal(s) * 0.05)(B, S, D)),
            "w1": _w((lambda *s: _rng.normal(s) * 0.05)(D, Dff)),
            "w2": _w((lambda *s: _rng.normal(s) * 0.05)(Dff, D)),
        }
    _B_in = _B_setup()

    return {
        "A_x": _A_in["x"],
        "A_wqkv": _A_in["wqkv"],
        "A_wo": _A_in["wo"],
        "B_x": _B_in["x"],
        "B_w1": _B_in["w1"],
        "B_w2": _B_in["w2"],
    }

def reference(A_x, A_wqkv, A_wo, B_x, B_w1, B_w2):
    def _A_ref(x, wqkv, wo):
        B, S, D = x.shape
        H = 32; Dh = D // H; W = 256
        qkv = (lambda x, *d: x.transpose(*d))((x @ wqkv).reshape(B, S, 3, H, Dh), 2, 0, 3, 1, 4)
        q, k, v = qkv[0], qkv[1], qkv[2]
        scores = jnp.einsum("bhqd,bhkd->bhqk", q, k) * (Dh ** -0.5)
        idx = jnp.arange(S)
        mask = (idx[:, None] - idx[None, :] >= 0) & (idx[:, None] - idx[None, :] < W)
        scores = jnp.where(mask[None, None], scores, -1e9)
        p = _softmax(scores, axis=-1)
        o = jnp.einsum("bhqk,bhkd->bhqd", p, v)
        return (lambda x, *d: x.transpose(*d))(o, 0, 2, 1, 3).reshape(B, S, D) @ wo

    def _B_ref(x, w1, w2):
        h = jnp.einsum("bsd,df->bsf", x, w1)
        zero = jnp.zeros_like(h)
        h = jnp.maximum(h, zero)
        return jnp.einsum("bsf,fd->bsd", h, w2)

    x = A_x
    h = x + _A_ref(_layernorm(x, axis=-1), A_wqkv, A_wo)
    h2 = h + _B_ref(_layernorm(h, axis=-1), B_w1, B_w2)
    return h2
```

```python
import functools
import math

import jax
import jax.numpy as jnp
from jax import lax
import jax.experimental.pallas as pl
import jax.experimental.pallas.tpu as pltpu

H = 32
W = 256
EPS = 1e-5
QB = 128
HB = QB // 2
SB = 32
NSB = QB // SB
NG = H // NSB
NPRO = 4
NHEAD = 6
UNROLL = 2
LAG = 12
F32 = jnp.float32
BF16 = jnp.bfloat16
U32 = jnp.uint32


def _acc(d, e, sign=1):
    for key, c in e.items():
        d[key] = d.get(key, 0) + sign * c
        if d[key] == 0:
            del d[key]
    return d


class _Products:
    def __init__(self):
        self.prods = []

    def new(self, oform, xform):
        self.prods.append((xform, {}, oform))
        return len(self.prods) - 1

    @staticmethod
    def at(vec, slot):
        return {(i, slot): c for i, c in vec.items()}

    def index(self, n, k, t):
        p, q = (t + 1) % 3, (t + 2) % 3
        own = {(q, p): self.new({(n, q): 1}, {(k, p): 1}), (p, q): self.new({(n, p): 1}, {(k, q): 1})}
        return ({n: 1}, {k: 1}, t, own), {own[q, p]: 1, own[p, q]: -1}

    def pair(self, u, v):
        (ua, ux, t0, ud), (va, vx, t1, vd) = u, v
        t2 = 3 - t0 - t1
        g = self.new(_acc(self.at(ua, t1), self.at(va, t0)), _acc(self.at(vx, t0), self.at(ux, t1), -1))
        ma, mx = _acc(dict(ua), va, -1), _acc(dict(ux), vx)
        r1 = self.new(self.at(ma, t0), self.at(mx, t1))
        r2 = self.new(self.at(ma, t1), self.at(mx, t0))
        uv = {g: 1, r1: -1, ud[t2, t1]: -1, vd[t0, t2]: 1}
        vu = {g: 1, r2: -1, ud[t1, t2]: -1, vd[t2, t0]: 1}
        return uv, vu, (ma, mx, t2, {(t0, t1): r1, (t1, t0): r2})

    def weigh(self, weight, prods):
        for r, c in prods.items():
            _acc(self.prods[r][1], {weight: c})

    def finish(self):
        out = []
        for x, w, o in self.prods:
            x = {key: -c if key[1] == 2 else c for key, c in x.items()}
            if all(c < 0 for c in x.values()):
                x, w = _acc({}, x, -1), _acc({}, w, -1)
            if all(c < 0 for c in w.values()):
                w, o = _acc({}, w, -1), _acc({}, o, -1)
            out.append((tuple(sorted(x.items())), tuple(sorted(w.items())), o))
        return out


def _square():
    s, types, cols = _Products(), (0, 1, 2, 0, 1), (1, 0, 2, 3, 4)
    idx, y, diff = [], {}, {}
    for i, t in enumerate(types):
        u, y[i, i] = s.index(cols[i], i, t)
        idx.append(u)
    for i in range(5):
        for j in range(5):
            if types[j] == (types[i] + 1) % 3:
                y[i, j], y[j, i], diff[i, j] = s.pair(idx[i], idx[j])
    for i, j, k in ((0, 1, 3), (1, 2, 4)):
        mk, km, _ = s.pair(diff[i, j], idx[k])
        y[i, k], y[k, i] = _acc(mk, y[j, k]), _acc(km, y[k, j], -1)
    for (i, j), prods in y.items():
        s.weigh((j, cols[i]), prods)
    return s.finish()


def _strassen(cells, singles):
    s = _Products()
    for (n0, k0), (n1, k1), t in cells:
        u, uu = s.index(n0, k0, t)
        v, vv = s.index(n1, k1, (t + 1) % 3)
        uv, vu, _ = s.pair(u, v)
        for n, k, prods in ((n0, k0, uu), (n1, k1, vv), (n0, k1, uv), (n1, k0, vu)):
            s.weigh((k, n), prods)
    for n, k, t in singles:
        s.weigh((k, n), s.index(n, k, t)[1])
    return s.finish()


ORDER40 = (35, 23, 0, 20, 19, 22, 21, 11, 34, 2, 6, 36, 26, 14, 29, 24, 38, 13, 10, 1,
           25, 30, 15, 12, 28, 8, 7, 27, 37, 17, 39, 31, 9, 32, 33, 18, 16, 4, 3, 5)
ORDER18 = (12, 10, 17, 1, 6, 4, 13, 9, 3, 11, 16, 2, 5, 15, 0, 7, 14, 8)
ORDER58 = (35, 6, 0, 23, 20, 5, 43, 19, 50, 21, 22, 11, 34, 26, 36, 45, 29, 14, 49, 42,
           52, 24, 38, 28, 25, 1, 8, 56, 13, 15, 10, 30, 12, 55, 44, 46, 39, 17, 32, 37,
           27, 53, 51, 7, 54, 4, 57, 31, 9, 33, 47, 16, 48, 18, 40, 3, 2, 41)
NWF = 8 * 40 + 2 * 18


def _add(terms):
    sign = 1 if any(c > 0 for c, _ in terms) else -1
    terms = sorted(terms, key=lambda t: -t[0] * sign)
    out = terms[0][1]
    for c, v in terms[1:]:
        out = out + v if c == sign else out - v
    return sign, out


def _total(terms):
    sign, out = _add(terms)
    return out if sign > 0 else -out


def _pack(x):
    return pltpu.bitcast(x.astype(BF16), U32)


def _dot(a, b, transposed=False):
    dims = (((1,), (1 if transposed else 0,)), ((), ()))
    return lax.dot_general(a, b, dims, preferred_element_type=F32)


def _lanes(c):
    return slice(c * 128, (c + 1) * 128)


def _half(n):
    return slice(n * HB, (n + 1) * HB)


class _Rows:
    def __init__(self, ref, n, rows, back):
        if isinstance(n, int):
            self.ref, self.base = ref, n * rows
        else:
            start = pl.multiple_of((n - back) * rows, rows)
            self.ref, self.base = ref.at[pl.ds(start, (back + 1) * rows)], back * rows

    def index(self, idx):
        rows, rest = (idx[0], idx[1:]) if isinstance(idx, tuple) else (idx, ())
        if isinstance(rows, slice):
            return (slice(self.base + rows.start, self.base + rows.stop),) + rest
        return (self.base + rows,) + rest

    def __getitem__(self, idx):
        return self.ref[self.index(idx)]

    def __setitem__(self, idx, value):
        self.ref[self.index(idx)] = value


def _kernel(x_hbm, wqkv_hbm, wo_hbm, w1_hbm, w2_hbm, y_hbm,
            x_s, wqkv_s, wo_s, w1_s, w2_s, y_s,
            wf_s,
            xf_s,
            q_s, k_s,
            vt_s,
            sc_s, p_s,
            ot_s, o_s,
            h_s,
            f_s,
            acc_s,
            msk_s, zero_s, sem_in, sem_out):
    S, D = x_s.shape
    Dh = D // H
    GW = NSB * Dh
    DT = D // 128
    NB = S // QB
    scale = Dh ** -0.5 * math.log2(math.e)
    opt = {}

    views = {}

    def block(ref, n, rows, back=0):
        key = (id(ref), n if isinstance(n, int) else id(n))
        if key not in views:
            views[key] = (_Rows(ref, n, rows, back), n)
        return views[key][0]

    loads = {}

    def load(name, src, dst, idx=slice(None)):
        loads[name] = pltpu.make_async_copy(src.at[idx], dst.at[idx], sem_in.at[len(loads)])

    def load_x(name, lo, hi):
        load(name, x_hbm, x_s, pl.ds(lo * QB, (hi - lo) * QB))

    def load_qkv(name, c, lo, hi):
        load(name, wqkv_hbm, wqkv_s, (slice(None), pl.ds(lo, hi - lo), pl.ds(c * D, D)))

    cut, early = 96, 3
    load_x('x0', 0, 2)
    load_qkv('q0', 0, 0, cut)
    load_qkv('q1', 0, cut, 128)
    load_x('x1', 2, NPRO)
    load_qkv('k0', 1, 0, cut)
    load_qkv('k1', 1, cut, 128)
    load_qkv('v', 2, 0, 128)
    load_x('x2', NPRO, NPRO + early + 2)
    load('o', wo_hbm, wo_s)
    load('f1', w1_hbm, w1_s)
    load('f2', w2_hbm, w2_s)
    load_x('x3', NPRO + early + 2, NB)
    ends = (0, NB - NHEAD, NB - 1, NB)
    stores = [pltpu.make_async_copy(y_s.at[rows], y_hbm.at[rows], sem_out.at[i])
              for i in range(3) for rows in [pl.ds(ends[i] * QB, (ends[i + 1] - ends[i]) * QB)]]
    for copy in loads.values():
        copy.start()

    def touch(i, carry):
        for ref in (wf_s, q_s, k_s, ot_s, o_s, h_s, f_s, p_s, sc_s, acc_s, xf_s):
            ref[pl.ds(pl.multiple_of(i * 8, 8), 8), 0:128] = jnp.zeros((8, 128), ref.dtype)
        for ref in (vt_s, msk_s):
            ref[i] = jnp.zeros(ref.shape[1:], ref.dtype)
        zero_s[i] = 0
        return carry
    lax.fori_loop(0, 2, touch, 0)

    lane = lax.broadcasted_iota(jnp.int32, (8, 128), 1)
    sub = lax.broadcasted_iota(jnp.int32, (8, 128), 0)
    for hd in range(H):
        msk_s[hd] = jnp.where((lane - hd * Dh % 128) % 128 < Dh, U32(0xFFFFFFFF), U32(0))
    for a in range(2):
        row = 16 * a + 2 * sub
        m = (jnp.where(row <= lane % SB, U32(0x0000FFFF), U32(0))
             | jnp.where(row + 1 <= lane % SB, U32(0xFFFF0000), U32(0)))
        msk_s[H + a] = m
        msk_s[H + 2 + a] = ~m
    causal = (lax.broadcasted_iota(jnp.int32, (SB, 128), 0)
              <= lax.broadcasted_iota(jnp.int32, (SB, 128), 1) % SB)
    quarter = {rows: lax.broadcasted_iota(jnp.int32, (rows, 128), 1) // SB for rows in (SB // 2, HB)}
    left = {rows: q < 2 for rows, q in quarter.items()}
    first = {rows: q == 0 for rows, q in quarter.items()}
    third = {rows: q == 2 for rows, q in quarter.items()}
    top4 = sub < 4

    zero = zero_s[0]
    always = sub >= zero
    ties, recent = [], []

    def tie(vals, delay):
        if delay:
            vals = [v if v.dtype == U32 else pltpu.bitcast(v, U32) for v in vals]
            ties.append((delay, functools.reduce(jnp.bitwise_or, vals)))

    def tied(w):
        due = [v for d, v in ties if d <= 1]
        ties[:] = [(d - 1, v) for d, v in ties if d > 1]
        if not due:
            return w
        head = jnp.where(always, w[:8], functools.reduce(jnp.bitwise_or, due))
        return jnp.concatenate([head, w[8:]], axis=0)

    def released(w):
        if not recent:
            return w
        keep = lax.broadcasted_iota(jnp.int32, w.shape, 0) >= zero
        return jnp.where(keep, w, jnp.concatenate(recent * (w.shape[1] // 128), axis=1))

    def call(fn):
        return [(0, lambda: (fn(), None)[1])]

    def wait(*names):
        return sum((call(loads.pop(name).wait) for name in names), [])

    square = _square()
    stages = {
        'q': (square, wqkv_s, 0, 0),
        'k': (square, wqkv_s, 0, DT),
        'v': (square, wqkv_s, 0, 2 * DT),
        'o': (square, wo_s, 0, 0),
        'f1a': (square, w1_s, 0, 0),
        'f1b': (square, w1_s, 0, DT),
        'f1c': (_strassen([((0, 0), (1, 1), 0), ((0, 2), (1, 3), 2)], [(0, 4, 1), (1, 4, 1)]), w1_s, 0, 2 * DT),
        'f2a': (square, w2_s, 0, 0),
        'f2b': (square, w2_s, DT, 0),
        'f2c': (_strassen([((0, 0), (1, 1), 0), ((2, 0), (3, 1), 0)], [(4, 0, 0), (4, 1, 1)]), w2_s, 2 * DT, 0),
    }
    wbase, count = {}, 0
    for name, stage in stages.items():
        wbase[name] = count
        count += len(stage[0])

    def weight_tasks(*names):
        parts = 14

        def run(name, r, part):
            scheme, w_ref, k0, n0 = stages[name]
            raw = lambda k, n: w_ref[k0 + k, r:r + 16, _lanes(n0 + n)]
            tile = functools.cache(lambda k, n: raw(k, n).astype(F32))
            order = sorted(range(len(scheme)),
                           key=lambda i: (len(scheme[i][2]) > 1, sorted({n for n, _ in scheme[i][2]})))
            done = []
            for a, i in enumerate(order):
                if a * parts // len(scheme) == part:
                    wform = scheme[i][1]
                    done.append((slice(r // 2, r // 2 + 8), _lanes(wbase[name] + i)))
                    if len(wform) == 1:
                        wf_s[done[-1]] = pltpu.bitcast(raw(*wform[0][0]), U32)
                    else:
                        wf_s[done[-1]] = _pack(_total([(c, tile(*kn)) for kn, c in wform]))
            if name != 'q':
                tie([wf_s[where] for where in done], 10)
        return [(0, functools.partial(run, name, r, part))
                for name in names for r in range(0, 128, 16) for part in range(parts)]

    def combine(tile):
        def build(xform):
            terms = [(c, tile(k, slot)) for (k, slot), c in xform]
            return _total(terms[:1] + terms[:0:-1]).astype(BF16)
        return build

    def normed(col):
        return combine(lambda k, slot: pltpu.bitcast(wf_s[:, _lanes(col + slot * DT + k)], F32))

    def product_tasks(emit, *groups):
        scheme = [(xform, [(wbase[name] + i, lhs) for name, lhs in group], oform) for group in groups
                  for i, (xform, _, oform) in enumerate(stages[group[0][0]][0])]
        scheme = [scheme[i] for i in {18: ORDER18, 40: ORDER40, 58: ORDER58}[len(scheme)]]
        last, uses, sums = {}, {}, {}
        for t, (_, _, oform) in enumerate(scheme):
            for key in oform:
                last[key[0]] = t
                uses.setdefault(key, []).append(t)

        def fetch(key):
            c, y = sums[key]
            return c, (acc_s[:, y] if isinstance(y, slice) else y)

        def run(t):
            xform, operands, oform = scheme[t]
            y = functools.reduce(jnp.add, [
                _dot(lhs(xform), pltpu.bitcast(tied(wf_s[:, _lanes(w)]), BF16)) for w, lhs in operands])

            def epilogue():
                recent[:] = [pltpu.bitcast(y[:8], U32)]
                for key, c in oform.items():
                    sums[key] = _add([fetch(key), (c, y)]) if key in sums else (c, y)
                for n in sorted(n for n in last if last[n] == t):
                    s0, s1, s2 = (fetch((n, slot)) for slot in range(3))
                    for slot in range(3):
                        del sums[n, slot]
                    emit(n, [s1, (-s2[0], s2[1])], [s2, (-s0[0], s0[1])])
                if t + 1 < len(scheme):
                    need = scheme[t + 1][2]
                    live = [key for key, (_, v) in sums.items() if not isinstance(v, slice) and key not in need]
                    live.sort(key=lambda key: next((u for u in uses[key] if u > t), last[key[0]]))
                    for key in live[max(0, 3 - len(need)):]:
                        where = _lanes(key[0] * 3 + key[1])
                        acc_s[:, where] = sums[key][1]
                        sums[key] = (sums[key][0], where)
            return epilogue
        return [(len(prod[1]), functools.partial(run, t)) for t, prod in enumerate(scheme)]

    def norm_tasks(n, col):
        hb, mean, mul = block(h_s, n, QB), {}, {}

        def pace(v, r):
            if r < HB and r % 16 == 0:
                tie([jnp.broadcast_to(v, (8, 128))], opt['norm_tie'])

        def mean_pass(r):
            mean[r] = jnp.sum(hb[r:r + 8], axis=-1, keepdims=True) * (1.0 / D)
            pace(mean[r], r)

        def var_pass(r):
            centred = hb[r:r + 8] - mean[r]
            mul[r] = lax.rsqrt(jnp.sum(centred * centred, axis=-1, keepdims=True) * (1.0 / D) + EPS)
            pace(mul[r], r)

        def norm_pass(r):
            top, bottom = ((hb[a:a + 8] - mean[a]) * mul[a] for a in (r, HB + r))
            for slot, y in enumerate((top, bottom, top + bottom)):
                lo = (col + slot * DT) * 128
                wf_s[r:r + 8, lo:lo + D] = pltpu.bitcast(y, U32)

        out, skew = [], opt['norm_skew']
        for a in range(HB // 8 + 2 * skew):
            for b, fn, offsets in ((a, mean_pass, (0, HB)), (a - skew, var_pass, (0, HB)),
                                   (a - 2 * skew, norm_pass, (0,))):
                if 0 <= b < HB // 8:
                    out += [(0, functools.partial(fn, 8 * b + off)) for off in offsets]
        return out

    def x_col(n):
        return NWF + (1 + n % NPRO) * 3 * DT

    def norm1_tasks(n):
        def widen(r):
            w = released(pltpu.bitcast(x_s[r:r + 16], U32))
            h_s[r:r + 16] = pltpu.bitcast(w, BF16).astype(F32)
        if n >= NB:
            return []
        return ([(0, functools.partial(widen, n * QB + r + off)) for r in range(0, HB, 16) for off in (0, HB)]
                + norm_tasks(n, x_col(n)))

    def group_tiles(g):
        return g * GW // 128, ((g + 1) * GW - 1) // 128

    straddling = [g for g in range(NG) if group_tiles(g)[0] != group_tiles(g)[1]]
    x_slot = {prod[0]: i for i, prod in enumerate(square)}

    def proj_tasks(n, name):
        done = set()

        def emit(c, top, bottom):
            y = jnp.concatenate([_total(top), _total(bottom)], axis=0)
            done.add(c)
            if name == 'q':
                q_s[_half(n), _lanes(c)] = _pack(y * scale)
            elif name == 'k':
                k_s[_half(n), _lanes(c)] = _pack(y)
                for i, g in enumerate(straddling):
                    t0, t1 = group_tiles(g)
                    if c in (t0, t1) and t0 in done and t1 in done:
                        upper = lax.broadcasted_iota(jnp.int32, (HB, 128), 1) >= g * GW % 128
                        k_s[_half(n), _lanes(DT + i)] = jnp.where(
                            upper, k_s[_half(n), _lanes(t0)], k_s[_half(n), _lanes(t1)])
            else:
                vt = y.T
                for a in range(16):
                    pair, pos = divmod(16 * c + a, 5)
                    t, hd = vt[8 * a:8 * a + 8], n * H + 2 * pair
                    if pos < 2:
                        vt_s[hd, 8 * pos:8 * pos + 8] = t
                    elif pos == 2:
                        vt_s[hd, 16:24] = jnp.where(top4, t, 1.0)
                        vt_s[hd + 1, 0:8] = jnp.where(top4, 1.0, t)
                    else:
                        vt_s[hd + 1, 8 * pos - 16:8 * pos - 8] = t
                tie([t], 36)

        def lhs(xform):
            slot = n % NPRO
            where = (slice(slot * HB // 2, (slot + 1) * HB // 2), _lanes(x_slot[xform]))
            if name != 'q':
                return pltpu.bitcast(xf_s[where], BF16)
            y = normed(x_col(n))(xform)
            xf_s[where] = pltpu.bitcast(y, U32)
            return y
        return product_tasks(emit, [(name, lhs)])

    def out_proj_tasks(n):
        hb, ob = block(h_s, n, QB), block(o_s, n, 3 * HB)

        def emit(c, *halves):
            for a, terms in enumerate(halves):
                hb[_half(a), _lanes(c)] = _total(terms + [(1, hb[_half(a), _lanes(c)])])
        return product_tasks(emit, [('o', combine(lambda k, slot: ob[_half(slot), _lanes(k)]))])

    def ffn1_tasks(part):
        def emit(c, *halves):
            top, bottom = (jnp.maximum(_total(terms), 0.0) for terms in halves)
            for slot, y in enumerate((top, bottom, top + bottom)):
                f_s[_half(slot), _lanes(DT * part + c)] = y
        return product_tasks(emit, [('f1' + 'abc'[part], normed(NWF))])

    def ffn2_tasks(n):
        hb, yb = block(h_s, n, QB), block(y_s, n, QB)

        def emit(c, *halves):
            for a, terms in enumerate(halves):
                y = _total(terms + [(1, hb[_half(a), _lanes(c)])])
                yb[_half(a), _lanes(c)] = y.astype(y_s.dtype)

        def lhs(k0):
            return combine(lambda k, slot: f_s[_half(slot), _lanes(k0 + k)])
        return product_tasks(emit, [('f2a', lhs(0)), ('f2b', lhs(DT))], [('f2c', lhs(2 * DT))])

    NS = W // SB

    def first_slab(n, j):
        return max(0, NS - j - n * NSB) if isinstance(n, int) else 0

    def scores(n, g, j):
        qb, rows = block(q_s, n, HB), slice(j * SB // 2, (j + 1) * SB // 2)
        parts = []
        for l in range(NSB):
            hd = g * NSB + (l - j) % NSB
            t0, t1 = hd * Dh // 128, ((hd + 1) * Dh - 1) // 128
            q = qb[rows, _lanes(t0)]
            if t0 != t1:
                q = pick(left, qb[rows, _lanes(t1)], q)
            parts.append(q & jnp.concatenate([msk_s[hd]] * 2, axis=0))
        q = pltpu.bitcast(jnp.concatenate(parts, axis=0), BF16)
        b0 = first_slab(n, j)
        col = DT + straddling.index(g) if g in straddling else group_tiles(g)[0]
        keys = block(k_s, n, HB, 2)[slice(((j + b0) * SB - W) // 2, (j + 1) * SB // 2), _lanes(col)]
        s = _dot(pltpu.bitcast(keys, BF16), q, True)
        if b0 == 0:
            inner, edge = s[SB:-SB], lax.select(causal, s[-SB:], s[:SB])
        else:
            inner, edge = s[:-SB] if b0 < NS else None, jnp.where(causal, s[-SB:], -jnp.inf)
        s = jnp.concatenate([inner, edge], axis=0) if b0 < NS else edge
        sc_s[0:s.shape[0], _lanes(j % 2)] = s
        return jnp.max(s, axis=0, keepdims=True)

    def p_rows(g, lo, hi):
        return slice((g % 4 * W + lo * SB) // 2, (g % 4 * W + hi * SB) // 2)

    def exponentiate(m, n, g, j):
        count = min(NS, NS + 1 - first_slab(n, j))
        p_s[p_rows(g, 0, count), _lanes(j)] = _pack(jnp.exp2(sc_s[0:count * SB, _lanes(j % 2)] - m))

    def probs(n, g, j, lo, hi):
        b0 = first_slab(n, j)
        if not b0 <= lo <= NS:
            return None
        if b0:
            return p_s[p_rows(g, lo - b0, hi - b0), _lanes(j)]
        if 0 < lo < NS:
            return p_s[p_rows(g, lo - 1, hi - 1), _lanes(j)]
        m = H if lo else H + 2
        return p_s[p_rows(g, NS - 1, NS), _lanes(j)] & msk_s[m:m + 2].reshape(SB // 2, 128)

    def pick(mask, a, b):
        if a is None and b is None:
            return None
        rows = (b if a is None else a).shape[0]
        none = jnp.zeros((rows, 128), U32)
        return lax.select(mask[rows], none if a is None else a, none if b is None else b)

    def weighted_values(n, g, i, a):
        cuts = (NSB, 2 * NSB) if a == 1 and first_slab(n, 0) == 0 else range(NSB * a, NSB * (a + 1) + 1)
        p = []
        for lo, hi in zip(cuts, cuts[1:]):
            src = [probs(n, g, j, lo - j, hi - j) for l in range(NSB) for j in [(l - i) % NSB]]
            p.append(pick(left, pick(first, src[0], src[1]), pick(third, src[2], src[3])))
        p = pltpu.bitcast(jnp.concatenate(p, axis=0), BF16)
        return _dot(block(vt_s, n, H, 2)[(a - 2) * H + g * NSB + i], p)

    def normalise(o, shared, n, g, i):
        den = o[0:1] if i % 2 else o[20:21]
        inv = pl.reciprocal(den, approx=True)
        o = o * (inv * (2.0 - den * inv))
        if i:
            o = pltpu.roll(o, 128 - SB * i, 1)
        r = g * GW + i // 2 * 2 * Dh
        if i % 2 == 0:
            ot_s[r:r + 16] = o[0:16]
            return o[16:24]
        ot_s[r + 16:r + 24] = jnp.where(top4, shared, o[0:8])
        ot_s[r + 24:r + 40] = o[8:24]
        for c in range(DT):
            if (c * 128 + 127) // (2 * Dh) == (g * NSB + i) // 2:
                complete.append((n, c))
        return shared

    complete, reading = [], []

    def untranspose():
        while complete and not reading:
            n, c = complete.pop(0)
            y, ob = ot_s[_lanes(c)].T, block(o_s, n, 3 * HB)
            ob[0:QB, _lanes(c)] = y
            ob[_half(2), _lanes(c)] = y[:HB] + y[HB:]

    pending, waits = [], []

    def tick():
        ready = [fn for d, fn in pending if d <= 0]
        pending[:] = [(d - 1, fn) for d, fn in pending if d > 0]
        for fn in ready:
            fn()

    def run(task):
        epilogue = task[1]()
        if task[0]:
            tick()
        if epilogue is not None:
            pending.append((opt['defer'] - 1, epilogue))

    def flush():
        while pending:
            tick()

    def weave(a, b, skip=0):
        out, a = a[:skip], a[skip:]
        n, k = sum(t[0] > 0 for t in a), 0
        for t in a:
            out.append(t)
            if t[0]:
                out += b[-(-k * len(b) // n):-(-(k + 1) * len(b) // n)]
                k += 1
        return out

    def mix(block_of, step0, value0, value1, delay, cost, dense, state):
        m, o, shared = state
        work, done, due = sum(t[0] for t in dense), 0, 0

        def unit(s):
            n = block_of(s // H)
            if isinstance(n, int) and not 0 <= n < NB:
                return None
            return n, s % H // NSB, s % NSB

        nxt, fresh = value0, unit(value0 - 1)
        for s, c in enumerate(cost, step0):
            head = None
            if nxt <= s - delay and nxt < value1:
                head, nxt = unit(nxt), nxt + 1
            if fresh and (head or delay == 0):
                shared = normalise(o, shared, *fresh)
            fresh = head
            untranspose()
            while waits:
                waits.pop(0)()
            m_next = scores(*unit(s)) if unit(s) else None
            due += c
            batch = []
            while dense and (dense[0][0] == 0 or (done + dense[0][0] / 2) * sum(cost) <= work * due):
                done += dense[0][0]
                batch.append(dense.pop(0))
            todo = [a for a in range(3) if head and not (isinstance(head[0], int) and head[0] - 2 + a < 0)]
            size, pos, placed, sums = sum(t[0] for t in batch), 0, -opt['gap'], []

            def place():
                y = weighted_values(*head, todo.pop(0))
                sums[:] = [sums[0] + y if sums else y]
            for task in batch:
                if (todo and task[0] and pos >= placed + opt['gap']
                        and pos >= size * (3 - len(todo)) / 3 + opt['shift']):
                    place()
                    placed = pos
                pos += task[0]
                run(task)
            while todo:
                place()
            o = sums[0] if sums else o
            if unit(s - 1):
                exponentiate(m, *unit(s - 1))
            m = m_next
        flush()
        ties.clear()
        recent.clear()
        return m, o, shared

    def projs(names, lo, hi):
        return sum((proj_tasks(n, name) for n in range(lo, hi) for name in names), [])

    def ffn_tasks(n, nxt):
        proj = out_proj_tasks(nxt)
        if not isinstance(n, int):
            proj = call(lambda: reading.append(n)) + proj + call(reading.clear)
        return (ffn1_tasks(0) + ffn1_tasks(1) + proj + ffn1_tasks(2)
                + weave(ffn2_tasks(n), norm_tasks(nxt, NWF), opt['defer'] + opt['norm_start']))

    opt.update(defer=2, norm_tie=0, norm_skew=1, shift=0, gap=3)
    wq, wk = weight_tasks('q'), weight_tasks('k')
    part = len(wq) * cut // 128
    start = wait('x0') + norm1_tasks(0) + norm1_tasks(1) + wait('q0') + wq[:part] + wait('q1') + wq[part:]
    start += call(ties.clear) + projs('q', 0, 1) + wait('x1')
    for n in range(1, NPRO - 1):
        start += weave(projs('q', n, n + 1), norm1_tasks(n + 1))
    start += wait('k0') + weave(projs('q', NPRO - 1, NPRO), wk[:part]) + wait('k1') + wk[part:] + call(ties.clear)
    start += projs('k', 0, NPRO - 1) + wait('v') + weave(projs('k', NPRO - 1, NPRO), weight_tasks('v'))
    start += projs('v', 0, NPRO - 1) + wait('x2', 'o') + weave(projs('v', NPRO - 1, NPRO), norm1_tasks(NPRO))
    for task in start + call(flush):
        run(task)

    qkv = [weave(projs('qvk', n, n + 1), norm1_tasks(n + 1), len(square)) for n in range(NPRO, NB)]
    dense = weave(sum(qkv[:early], []), weight_tasks('o'))
    dense[-20:-20] = call(functools.partial(waits.extend, [fn for _, fn in wait('f1', 'f2', 'x3')]))
    rest = (sum(qkv[early:-3], []) + out_proj_tasks(0)
            + weave(sum(qkv[-3:], []), norm_tasks(0, NWF), opt['defer']))
    part = len(rest) * 85 // 100
    dense += weave(rest[:part], weight_tasks('f1a', 'f1b', 'f1c', 'f2a', 'f2b', 'f2c')) + rest[part:]
    cost = [NS + 1 - first_slab(s // H, s % NSB) + (s < 2 * H) for s in range(NHEAD * H)]
    state = (jnp.zeros((1, 128), F32), jnp.zeros((24, 128), F32), jnp.zeros((8, 128), F32))
    state = mix(lambda n: n, 0, 0, NHEAD * H - LAG, LAG, cost, dense, state)

    def steady(i, state):
        ffn = [i * UNROLL + d for d in range(UNROLL + 1)]
        att = {d: NHEAD + i * UNROLL + d for d in range(-1, UNROLL)}
        dense = sum((ffn_tasks(*ffn[d:d + 2]) for d in range(UNROLL)), [])
        return mix(att.get, 0, -LAG, UNROLL * H - LAG, LAG, [1] * (UNROLL * H), dense, state)
    opt.update(defer=4, norm_tie=24, norm_skew=2, norm_start=5, shift=1, gap=2)
    state = lax.fori_loop(0, (NB - NHEAD) // UNROLL, steady, state)
    stores[0].start()

    opt.update(defer=3, norm_tie=32, norm_start=0)
    dense = sum((ffn_tasks(n, n + 1) for n in range(NB - NHEAD, NB - 1)), [])
    dense += call(flush) + call(stores[1].start)
    dense += ffn1_tasks(0) + ffn1_tasks(1) + ffn1_tasks(2) + ffn2_tasks(NB - 1)
    mix(lambda n: n, NB * H, NB * H - LAG, NB * H, 0, [1] * (LAG + 1) + [20], dense, state)
    stores[2].start()
    for copy in stores:
        copy.wait()


@jax.jit
def pallas_sequential_preLN__sliding_block__dense_activation_relu__prompt_kernel(
    A_x: jax.Array,
    A_wqkv: jax.Array,
    A_wo: jax.Array,
    B_x: jax.Array,
    B_w1: jax.Array,
    B_w2: jax.Array,
):
    del B_x
    B, S, D = A_x.shape
    Dff = B_w1.shape[1]
    assert (B, S, D, Dff) == (1, 2048, 640, 1536)
    NB = S // QB
    weights = [w.reshape(w.shape[0] // 128, 128, w.shape[1]) for w in (A_wqkv, A_wo, B_w1, B_w2)]
    hbm = pl.BlockSpec(memory_space=pl.ANY)
    out = pl.pallas_call(
        _kernel,
        in_specs=[hbm] * 5,
        out_specs=hbm,
        out_shape=jax.ShapeDtypeStruct((S, D), A_x.dtype),
        scratch_shapes=[
            pltpu.VMEM((S, D), A_x.dtype),
            *[pltpu.VMEM(w.shape, w.dtype) for w in weights],
            pltpu.VMEM((S, D), A_x.dtype),
            pltpu.VMEM((HB, NWF * 128 + (NPRO + 1) * 3 * D), U32),
            pltpu.VMEM((NPRO * HB // 2, 41 * 128), U32),
            pltpu.VMEM((S // 2, D), U32),
            pltpu.VMEM((S // 2, D + 4 * 128), U32),
            pltpu.VMEM((NB * H, 24, 128), F32),
            pltpu.VMEM((W, 3 * 128), F32),
            pltpu.VMEM((4 * W // 2, (NSB + 1) * 128), U32),
            pltpu.VMEM((D, QB), F32),
            pltpu.VMEM((NB * 3 * HB, D), F32),
            pltpu.VMEM((S, D), F32),
            pltpu.VMEM((3 * HB, Dff + 128), F32),
            pltpu.VMEM((HB, 3 * D), F32),
            pltpu.VMEM((H + 4, 8, 128), U32),
            pltpu.SMEM((2,), jnp.int32),
            pltpu.SemaphoreType.DMA((12,)),
            pltpu.SemaphoreType.DMA((3,)),
        ],
        compiler_params=pltpu.CompilerParams(vmem_limit_bytes=100 * 2**20),
        name="fused_block",
    )(A_x.reshape(S, D), *weights)
    return out.reshape(B, S, D)
```
